```python
import os as _os
_os.environ.setdefault("JAX_PLATFORMS", "cpu")
import jax
import jax.numpy as jnp

def _softmax(x, axis=-1):
    return jax.nn.softmax(x, axis=axis)
def _gelu(x):
    return jax.nn.gelu(x, approximate=True)
def _silu(x):
    return jax.nn.silu(x)
def _sigmoid(x):
    return jax.nn.sigmoid(x)
def _layernorm(x, axis=-1, eps=1e-5):
    m = jnp.mean(x, axis=axis, keepdims=True)
    v = jnp.var(x, axis=axis, keepdims=True)
    return (x - m) / jnp.sqrt(v + eps)
def _scatter_add(tgt, idx, src, axis=0):
    return tgt.at[idx].add(src)
def _segment_sum(src, seg, n):
    return jax.ops.segment_sum(src, seg, n)
class _Rng:
    def __init__(self, key):
        self._k = key
    def _next(self):
        self._k, sub = jax.random.split(self._k)
        return sub
    def normal(self, shape):
        return jax.random.normal(self._next(), shape, dtype=jnp.bfloat16)
    def randint(self, lo, hi, shape):
        return jax.random.randint(self._next(), shape, lo, hi, dtype=jnp.int32)
    def uniform(self, shape, lo=0.0, hi=1.0):
        return jax.random.uniform(self._next(), shape, jnp.bfloat16, lo, hi)
    def permutation(self, n):
        return jax.random.permutation(self._next(), n)


kernel_name = 'concat_heads__mha_block_cached__mha_block_cached__near_ridge'

def setup_inputs():
    _rng = _Rng(jax.random.key(int.from_bytes(__import__("os").urandom(4), "little")))
    _w = (lambda a: (lambda t: t.astype(jnp.bfloat16) if jnp.issubdtype(t.dtype, jnp.floating) else t)(jnp.asarray(a)))
    def _A_setup():
        B, Sq, D = 16, 80, 512
        H, Sk, Dh = 32, 80, 128
        return {
            "x": _w((lambda *s: _rng.normal(s) * 0.8)(B, Sq, D)),
            "k_cache": _w((lambda *s: _rng.normal(s) * 0.8)(B, H, Sk, Dh)),
            "v_cache": _w((lambda *s: _rng.normal(s) * 0.05)(B, H, Sk, Dh)),
            "wq": _w((lambda *s: _rng.normal(s) * 0.8)(D, H * Dh) * (D ** -0.5)),
            "wo": _w((lambda *s: _rng.normal(s) * 0.05)(H * Dh, D) * ((H * Dh) ** -0.5)),
        }
    _A_in = _A_setup()

    def _B_setup():
        B, Sq, D = 16, 80, 512
        H, Sk, Dh = 32, 80, 128
        return {
            "x": _w((lambda *s: _rng.normal(s) * 0.8)(B, Sq, D)),
            "k_cache": _w((lambda *s: _rng.normal(s) * 0.8)(B, H, Sk, Dh)),
            "v_cache": _w((lambda *s: _rng.normal(s) * 0.05)(B, H, Sk, Dh)),
            "wq": _w((lambda *s: _rng.normal(s) * 0.8)(D, H * Dh) * (D ** -0.5)),
            "wo": _w((lambda *s: _rng.normal(s) * 0.05)(H * Dh, D) * ((H * Dh) ** -0.5)),
        }
    _B_in = _B_setup()

    return {
        "A_x": _A_in["x"],
        "A_k_cache": _A_in["k_cache"],
        "A_v_cache": _A_in["v_cache"],
        "A_wq": _A_in["wq"],
        "A_wo": _A_in["wo"],
        "B_x": _B_in["x"],
        "B_k_cache": _B_in["k_cache"],
        "B_v_cache": _B_in["v_cache"],
        "B_wq": _B_in["wq"],
        "B_wo": _B_in["wo"],
    }

def reference(A_x, A_k_cache, A_v_cache, A_wq, A_wo, B_x, B_k_cache, B_v_cache, B_wq, B_wo):
    def _A_ref(x, k_cache, v_cache, wq, wo):
        B, Sq, D = x.shape
        H, Dh = 32, 128
        q = (lambda x, *d: x.transpose(*d))((x @ wq).reshape(B, Sq, H, Dh), 0, 2, 1, 3)
        scores = jnp.einsum("bhqd,bhkd->bhqk", q, k_cache) * (Dh ** -0.5)
        p = _softmax(scores, axis=-1)
        o = jnp.einsum("bhqk,bhkd->bhqd", p, v_cache)
        return (lambda x, *d: x.transpose(*d))(o, 0, 2, 1, 3).reshape(B, Sq, H * Dh) @ wo

    def _B_ref(x, k_cache, v_cache, wq, wo):
        B, Sq, D = x.shape
        H, Dh = 32, 128
        q = (lambda x, *d: x.transpose(*d))((x @ wq).reshape(B, Sq, H, Dh), 0, 2, 1, 3)
        scores = jnp.einsum("bhqd,bhkd->bhqk", q, k_cache) * (Dh ** -0.5)
        p = _softmax(scores, axis=-1)
        o = jnp.einsum("bhqk,bhkd->bhqd", p, v_cache)
        return (lambda x, *d: x.transpose(*d))(o, 0, 2, 1, 3).reshape(B, Sq, H * Dh) @ wo

    a = _A_ref(A_x, A_k_cache, A_v_cache, A_wq, A_wo)
    b = _B_ref(B_x, B_k_cache, B_v_cache, B_wq, B_wo)
    return jnp.concatenate([a, b], axis=-1)
```

```python
import jax
import jax.numpy as jnp
from jax import lax
import jax.experimental.pallas as pl
import jax.experimental.pallas.tpu as pltpu

B, SQ, D = 16, 80, 512
H, SK, DH = 32, 80, 128
G = 4
NG = H // G
NS = 2 * NG
M = B * SQ
GW = G * DH
SCALE = DH ** -0.5
MCQ = 640
MCO = 640
SKEW = 3
GS = 4
AHEAD = 2
XCH = 2
NQ = AHEAD + 1
NT = (((1,), (1,)), ((), ()))
bf = jnp.bfloat16
f32 = jnp.float32


def _kernel(xa, ka, va, wqa, woa, xb, kb, vb, wqb, wob, out_hbm,
            x_buf, k_buf, v_buf, wq_buf, wo_buf, q_buf, o_buf, acc, out_buf,
            sem_x, sem_k, sem_v, sem_wq, sem_wo, sem_out):
    srcs = ((xa, ka, va, wqa, woa), (xb, kb, vb, wqb, wob))
    XR = M // XCH

    def xa_copy(c):
        r = pl.ds(c * XR, XR)
        return pltpu.make_async_copy(xa.at[r], x_buf.at[0, r], sem_x.at[c])

    def xb_copy():
        return pltpu.make_async_copy(xb, x_buf.at[1], sem_x.at[XCH])

    def wq_copy(br_static, s, g):
        return pltpu.make_async_copy(srcs[br_static][3].at[:, pl.ds(g * GW, GW)], wq_buf.at[s], sem_wq.at[s])

    def kvo_copies(br_static, s, g):
        _, k, v, wq, wo = srcs[br_static]
        hs = pl.ds(g * G, G)
        return (
            pltpu.make_async_copy(k.at[:, hs], k_buf.at[s], sem_k.at[s]),
            pltpu.make_async_copy(v.at[:, hs], v_buf.at[s], sem_v.at[s]),
            pltpu.make_async_copy(wo.at[pl.ds(g * GW, GW), :], wo_buf.at[s], sem_wo.at[s]),
        )

    def issue_kvo(s):
        @pl.when(s < NG)
        def _():
            for c in kvo_copies(0, s, s):
                c.start()

        @pl.when(jnp.logical_and(s >= NG, s < NS))
        def _():
            for c in kvo_copies(1, s, s - NG):
                c.start()

    def issue_wq(t):
        @pl.when(t < NG)
        def _():
            wq_copy(0, t, t).start()

        @pl.when(t == NG)
        def _():
            xb_copy().start()

        @pl.when(jnp.logical_and(t >= NG, t < NS))
        def _():
            wq_copy(1, t, t - NG).start()

    def qproj_rows(s, r):
        br = s // NG
        slot = s % NQ
        q = jnp.dot(x_buf[br, r, :], wq_buf[s], preferred_element_type=f32)
        q_buf[slot, r, :] = (q * SCALE).astype(bf)

    def qproj(s):
        for c in range(M // MCQ):
            qproj_rows(s, slice(c * MCQ, (c + 1) * MCQ))

    def wait_wq(s):
        @pl.when(s == NG)
        def _():
            xb_copy().wait()
        wq_copy(0, s, 0).wait()

    def attn_oproj(s):
        br = s // NG
        g = s % NG
        slot = s % NQ
        heads = [(b, h) for b in range(B) for h in range(G)]
        groups = [heads[j:j + GS] for j in range(0, len(heads), GS)]
        n = len(groups)
        P = {}

        def qk(j):
            for (b, h) in groups[j]:
                q = q_buf[slot, b * SQ:(b + 1) * SQ, h * DH:(h + 1) * DH]
                k = k_buf[s, b, h]
                sc = lax.dot_general(q, k, NT, preferred_element_type=f32)
                m = jnp.max(sc, axis=-1, keepdims=True)
                p = jnp.exp(sc - m)
                l = jnp.sum(p, axis=-1, keepdims=True)
                P[(b, h)] = (p.astype(bf), l)

        def pv(j):
            for (b, h) in groups[j]:
                p, l = P.pop((b, h))
                v = v_buf[s, b, h]
                o = jnp.dot(p, v, preferred_element_type=f32)
                o_buf[b * SQ:(b + 1) * SQ, h * DH:(h + 1) * DH] = (
                    o * pl.reciprocal(l, approx=True)).astype(bf)

        for j in range(n + SKEW):
            if j < n:
                qk(j)
            if j - SKEW >= 0:
                pv(j - SKEW)

        for c in range(M // MCO):
            r = slice(c * MCO, (c + 1) * MCO)
            o = jnp.dot(o_buf[r, :], wo_buf[s], preferred_element_type=f32)
            new = jnp.where(g == 0, 0.0, acc[r, :]) + o
            acc[r, :] = new
            out_buf[br, r, :] = new.astype(bf)

    def wait_kvo(s):
        for c in kvo_copies(0, s, 0):
            c.wait()

    def finish(s):
        br = s // NG

        @pl.when(s % NG == NG - 1)
        def _():
            pltpu.make_async_copy(out_buf.at[br], out_hbm.at[:, pl.ds(pl.multiple_of(br * D, D), D)],
                                  sem_out.at[br]).start()

    wq_copy(0, 0, 0).start()
    for c in range(XCH):
        xa_copy(c).start()
    wq_copy(0, 0, 0).wait()
    xa_copy(0).wait()
    for t in range(1, AHEAD + 1):
        wq_copy(0, t, t).start()
    for c in kvo_copies(0, 0, 0):
        c.start()

    def pro0(c, carry):
        @pl.when(c > 0)
        def _():
            xa_copy(c).wait()
        qproj_rows(0, pl.ds(pl.multiple_of(c * XR, XR), XR))
        return carry
    if XCH == 1:
        qproj(0)
    else:
        lax.fori_loop(0, XCH, pro0, 0)

    def pro(s, carry):
        wait_wq(s)
        qproj(s)
        return carry
    if AHEAD > 1:
        lax.fori_loop(1, AHEAD, pro, 0)

    def main(s, carry):
        wait_kvo(s)
        wait_wq(s + AHEAD)
        issue_kvo(s + 1)
        issue_wq(s + 1 + AHEAD)
        attn_oproj(s)
        qproj(s + AHEAD)
        finish(s)
        return carry
    lax.fori_loop(0, NS - AHEAD, main, 0)

    def tail(s, carry):
        wait_kvo(s)
        issue_kvo(s + 1)
        attn_oproj(s)
        finish(s)
        return carry
    lax.fori_loop(NS - AHEAD, NS, tail, 0)

    for br in range(2):
        pltpu.make_async_copy(out_buf.at[br], out_hbm.at[:, pl.ds(br * D, D)], sem_out.at[br]).wait()


@jax.jit
def pallas_concat_heads__mha_block_cached__mha_block_cached__near_ridge_kernel(
    A_x, A_k_cache, A_v_cache, A_wq, A_wo, B_x, B_k_cache, B_v_cache, B_wq, B_wo,
):
    any_spec = pl.BlockSpec(memory_space=pl.ANY)
    out = pl.pallas_call(
        _kernel,
        out_shape=jax.ShapeDtypeStruct((M, 2 * D), bf),
        in_specs=[any_spec] * 10,
        out_specs=any_spec,
        scratch_shapes=[
            pltpu.VMEM((2, M, D), bf),
            pltpu.VMEM((NS, B, G, SK, DH), bf),
            pltpu.VMEM((NS, B, G, SK, DH), bf),
            pltpu.VMEM((NS, D, GW), bf),
            pltpu.VMEM((NS, GW, D), bf),
            pltpu.VMEM((NQ, M, GW), bf),
            pltpu.VMEM((M, GW), bf),
            pltpu.VMEM((M, D), f32),
            pltpu.VMEM((2, M, D), bf),
            pltpu.SemaphoreType.DMA((XCH + 1,)),
            pltpu.SemaphoreType.DMA((NS,)),
            pltpu.SemaphoreType.DMA((NS,)),
            pltpu.SemaphoreType.DMA((NS,)),
            pltpu.SemaphoreType.DMA((NS,)),
            pltpu.SemaphoreType.DMA((2,)),
        ],
        compiler_params=pltpu.CompilerParams(vmem_limit_bytes=110 * 1024 * 1024,
                                             disable_bounds_checks=True),
    )(A_x.reshape(M, D), A_k_cache, A_v_cache, A_wq, A_wo,
      B_x.reshape(M, D), B_k_cache, B_v_cache, B_wq, B_wo)
    return out.reshape(B, SQ, 2 * D)
```

```python
import jax
import jax.numpy as jnp
from jax import lax
import jax.experimental.pallas as pl
import jax.experimental.pallas.tpu as pltpu

B, SQ, D = 16, 80, 512
H, SK, DH = 32, 80, 128
G = 8
NG = H // G
NS = 2 * NG
M = B * SQ
GW = G * DH
SCALE = DH ** -0.5
MCQ = 640
OCH = (80, 80, 160, 320, 320, 160, 80, 80)
SKEW = 3
GS = 4
AHEAD = 2
NQ = 4 if G < 16 else 3
NOC = len(OCH)
OST = [sum(OCH[:i]) for i in range(NOC)]
assert sum(OCH) == M
NT = (((1,), (1,)), ((), ()))
bf = jnp.bfloat16
f32 = jnp.float32
PW = 4 * DH
XR = 320


def _kernel(xa, ka, va, wqa, woa, xb, kb, vb, wqb, wob, out_hbm,
            x_buf, k_buf, v_buf, wq_buf, wo_buf, q_buf, o_buf, acc, out_buf,
            sem_x, sem_p, sem_k, sem_v, sem_wq, sem_wo, sem_out, sem_f):
    srcs = ((xa, ka, va, wqa, woa), (xb, kb, vb, wqb, wob))

    def wait_for(dst, sem):
        pltpu.make_async_copy(dst, dst, sem).wait()

    def wq_copy(br_static, s, g):
        return pltpu.make_async_copy(srcs[br_static][3].at[:, pl.ds(g * GW, GW)], wq_buf.at[s], sem_wq.at[s])

    def kv_copies(br_static, s, g):
        _, k, v, wq, wo = srcs[br_static]
        hs = pl.ds(g * G, G)
        return (
            pltpu.make_async_copy(k.at[:, hs], k_buf.at[s], sem_k.at[s]),
            pltpu.make_async_copy(v.at[:, hs], v_buf.at[s], sem_v.at[s]),
        )

    def wo_copy(br_static, s, g):
        return pltpu.make_async_copy(srcs[br_static][4].at[pl.ds(g * GW, GW), :], wo_buf.at[s], sem_wo.at[s])

    def xb_copy():
        return pltpu.make_async_copy(xb, x_buf.at[1], sem_x.at[3])

    def issue_kvo(s):
        @pl.when(s < NG)
        def _():
            for c in kv_copies(0, s, s):
                c.start()
            wo_copy(0, s, s).start()

        @pl.when(jnp.logical_and(s >= NG, s < NS))
        def _():
            for c in kv_copies(1, s, s - NG):
                c.start()
            wo_copy(1, s, s - NG).start()

    def issue_wq(t):
        @pl.when(t < NG)
        def _():
            wq_copy(0, t, t).start()

        @pl.when(t == NG)
        def _():
            xb_copy().start()

        @pl.when(jnp.logical_and(t >= NG, t < NS))
        def _():
            wq_copy(1, t, t - NG).start()

    def qproj_piece(s, r, c0, c1):
        br = s // NG
        slot = s % NQ
        q = jnp.dot(x_buf[br, r, :], wq_buf[s, :, c0:c1], preferred_element_type=f32)
        q_buf[slot, r, c0:c1] = (q * SCALE).astype(bf)

    def qproj(s, c0=0, c1=GW):
        for c in range(M // MCQ):
            qproj_piece(s, slice(c * MCQ, (c + 1) * MCQ), c0, c1)

    def wait_wq(s):
        @pl.when(s == NG)
        def _():
            wait_for(x_buf.at[1], sem_x.at[3])
        wait_for(wq_buf.at[s], sem_wq.at[s])

    def out_copy(br, c):
        r = pl.ds(OST[c], OCH[c])
        return pltpu.make_async_copy(out_buf.at[br, r], out_hbm.at[r, pl.ds(pl.multiple_of(br * D, D), D)],
                                     sem_out.at[br * NOC + c])

    def attn(s):
        slot = s % NQ
        heads = [(b, h) for b in range(B) for h in range(G)]
        groups = [heads[j:j + GS] for j in range(0, len(heads), GS)]
        n = len(groups)
        P = {}

        def qk(j):
            for (b, h) in groups[j]:
                q = q_buf[slot, b * SQ:(b + 1) * SQ, h * DH:(h + 1) * DH]
                k = k_buf[s, b, h]
                sc = lax.dot_general(q, k, NT, preferred_element_type=f32)
                m = jnp.max(sc, axis=-1, keepdims=True)
                p = jnp.exp(sc - m)
                l = jnp.sum(p, axis=-1, keepdims=True)
                P[(b, h)] = (p.astype(bf), l)

        def pv(j):
            for (b, h) in groups[j]:
                p, l = P.pop((b, h))
                v = v_buf[s, b, h]
                o = jnp.dot(p, v, preferred_element_type=f32)
                r0 = pl.reciprocal(l, approx=True)
                o = o * (r0 * (2.0 - l * r0))
                o_buf[b * SQ:(b + 1) * SQ, h * DH:(h + 1) * DH] = o.astype(bf)

        for j in range(n + SKEW):
            if j < n:
                qk(j)
            if j - SKEW >= 0:
                pv(j - SKEW)

    def oproj(s):
        br = s // NG
        g = s % NG
        for c in range(NOC):
            r = slice(OST[c], OST[c] + OCH[c])
            o = jnp.dot(o_buf[r, :], wo_buf[s], preferred_element_type=f32)
            new = jnp.where(g == 0, 0.0, acc[r, :]) + o
            acc[r, :] = new
            out_buf[br, r, :] = new.astype(bf)

            @pl.when(g == NG - 1)
            def _():
                out_copy(br, c).start()

    def wait_kvo(s):
        wait_for(k_buf.at[s], sem_k.at[s])
        wait_for(v_buf.at[s], sem_v.at[s])
        wait_for(wo_buf.at[s], sem_wo.at[s])

    def x_piece(i):
        r = (pl.ds(0, XR), pl.ds(XR, XR), pl.ds(2 * XR, M - 2 * XR))[i]
        return pltpu.make_async_copy(xa.at[r], x_buf.at[0, r], sem_x.at[i])

    def wq_piece(i):
        lo, hi = ((0, PW), (PW, min(2 * PW, GW)), (2 * PW, GW))[i]
        return pltpu.make_async_copy(wqa.at[:, lo:hi], wq_buf.at[0, :, lo:hi], sem_p.at[i])

    def fence():
        pl.semaphore_signal(sem_f, 1)
        pl.semaphore_wait(sem_f, 1)

    first = [wq_piece(0), x_piece(0), x_piece(1), x_piece(2)]
    if GW > PW:
        first.append(wq_piece(1))
    if GW > 2 * PW:
        first.append(wq_piece(2))
    first.append(wq_copy(0, 1, 1))
    first.extend(kv_copies(0, 0, 0))
    first.append(wo_copy(0, 0, 0))
    if NG > 2:
        first.append(wq_copy(0, 2, 2))
    for cp in first:
        cp.start()
        fence()

    wq_piece(0).wait()

    def pro0(c, carry):
        r = pl.ds(pl.multiple_of(c * XR, XR), XR)
        wait_for(x_buf.at[0, r], sem_x.at[c])
        qproj_piece(0, r, 0, PW)
        return carry
    lax.fori_loop(0, 2, pro0, 0)

    x_piece(2).wait()
    if GW > PW:
        wq_piece(1).wait()
    qproj_piece(0, slice(2 * XR, M), 0, PW)
    if GW > PW:
        qproj(0, PW, min(2 * PW, GW))
    if GW > 2 * PW:
        wq_piece(2).wait()
    wait_for(wq_buf.at[1], sem_wq.at[1])
    if NG == 2:
        xb_copy().start()
        wq_copy(1, 2, 0).start()
    if GW > 2 * PW:
        qproj(0, 2 * PW, GW)
    qproj(1)

    def main(s, carry):
        wait_kvo(s)
        wait_wq(s + AHEAD)
        issue_kvo(s + 1)
        issue_wq(s + 1 + AHEAD)
        attn(s)
        qproj(s + AHEAD)
        oproj(s)
        return carry
    lax.fori_loop(0, NS - AHEAD, main, 0)

    def tail(s, carry):
        wait_kvo(s)
        issue_kvo(s + 1)
        attn(s)
        oproj(s)
        return carry
    lax.fori_loop(NS - AHEAD, NS, tail, 0)

    for br in range(2):
        for c in range(NOC):
            out_copy(br, c).wait()


@jax.jit
def pallas_concat_heads__mha_block_cached__mha_block_cached__near_ridge_kernel(
    A_x, A_k_cache, A_v_cache, A_wq, A_wo, B_x, B_k_cache, B_v_cache, B_wq, B_wo,
):
    any_spec = pl.BlockSpec(memory_space=pl.ANY)
    out = pl.pallas_call(
        _kernel,
        out_shape=jax.ShapeDtypeStruct((M, 2 * D), bf),
        in_specs=[any_spec] * 10,
        out_specs=any_spec,
        scratch_shapes=[
            pltpu.VMEM((2, M, D), bf),
            pltpu.VMEM((NS, B, G, SK, DH), bf),
            pltpu.VMEM((NS, B, G, SK, DH), bf),
            pltpu.VMEM((NS, D, GW), bf),
            pltpu.VMEM((NS, GW, D), bf),
            pltpu.VMEM((NQ, M, GW), bf),
            pltpu.VMEM((M, GW), bf),
            pltpu.VMEM((M, D), f32),
            pltpu.VMEM((2, M, D), bf),
            pltpu.SemaphoreType.DMA((4,)),
            pltpu.SemaphoreType.DMA((3,)),
            pltpu.SemaphoreType.DMA((NS,)),
            pltpu.SemaphoreType.DMA((NS,)),
            pltpu.SemaphoreType.DMA((NS,)),
            pltpu.SemaphoreType.DMA((NS,)),
            pltpu.SemaphoreType.DMA((2 * NOC,)),
            pltpu.SemaphoreType.REGULAR,
        ],
        compiler_params=pltpu.CompilerParams(vmem_limit_bytes=120 * 1024 * 1024,
                                             disable_bounds_checks=True,
                                             disable_semaphore_checks=True),
    )(A_x.reshape(M, D), A_k_cache, A_v_cache, A_wq, A_wo,
      B_x.reshape(M, D), B_k_cache, B_v_cache, B_wq, B_wo)
    return out.reshape(B, SQ, 2 * D)
```

```python
import jax
import jax.numpy as jnp
from jax import lax
import jax.experimental.pallas as pl
import jax.experimental.pallas.tpu as pltpu

B, SQ, D = 16, 80, 512
H, SK, DH = 32, 80, 128
G = 8
NG = H // G
NS = 2 * NG
M = B * SQ
GW = G * DH
SCALE = DH ** -0.5
MCQ = 640
OCH = (80, 80, 160, 320, 320, 160, 80, 80)
NOC = len(OCH)
OST = tuple(sum(OCH[:i]) for i in range(NOC))
GS = 4
SKEW = 3
AHEAD = 2
NQ = 4
NT = (((1,), (1,)), ((), ()))
bf = jnp.bfloat16
f32 = jnp.float32

PIECES = (("w", 0, 256), ("x", 0, 80), ("x", 80, 240), ("w", 256, 512), ("x", 240, 560), ("x", 560, 1280), ("w", 512, 1024))
PRO = (((0, 1), ((0, 80, 0, 256),)),
       ((2,), ((80, 240, 0, 256),)),
       ((3,), ((0, 240, 256, 512),)),
       ((4,), ((240, 560, 0, 512),)),
       ((5,), ((560, 1280, 0, 512),)),
       ((6,), ((0, 1280, 512, 1024),)))


def _kernel(xa, ka, va, wqa, woa, xb, kb, vb, wqb, wob, out_hbm,
            x_buf, k_buf, v_buf, wq_buf, wo_buf, q_buf, o_buf, acc, out_buf,
            sem_x, sem_p, sem_k, sem_v, sem_wq, sem_wo, sem_out, sem_f, once):
    srcs = ((xa, ka, va, wqa, woa), (xb, kb, vb, wqb, wob))

    def wait_for(dst, sem):
        pltpu.make_async_copy(dst, dst, sem).wait()

    def wq_copy(br, s, g):
        return pltpu.make_async_copy(srcs[br][3].at[:, pl.ds(g * GW, GW)], wq_buf.at[s], sem_wq.at[s])

    def kvo_copies(br, s, g):
        _, k, v, _, wo = srcs[br]
        hs = pl.ds(g * G, G)
        return (
            pltpu.make_async_copy(k.at[:, hs], k_buf.at[s], sem_k.at[s]),
            pltpu.make_async_copy(v.at[:, hs], v_buf.at[s], sem_v.at[s]),
            pltpu.make_async_copy(wo.at[pl.ds(g * GW, GW), :], wo_buf.at[s], sem_wo.at[s]),
        )

    def xb_copy():
        return pltpu.make_async_copy(xb, x_buf.at[1], sem_x)

    def piece(i):
        kind, lo, hi = PIECES[i]
        if kind == "x":
            return pltpu.make_async_copy(xa.at[lo:hi], x_buf.at[0, lo:hi], sem_p.at[i])
        return pltpu.make_async_copy(wqa.at[:, lo:hi], wq_buf.at[0, :, lo:hi], sem_p.at[i])

    def out_copy(br, c):
        r = pl.ds(OST[c], OCH[c])
        return pltpu.make_async_copy(out_buf.at[br, r], out_hbm.at[r, pl.ds(pl.multiple_of(br * D, D), D)],
                                     sem_out.at[br * NOC + c])

    def issue_kvo(s):
        @pl.when(s < NG)
        def _():
            for c in kvo_copies(0, s, s):
                c.start()

        @pl.when(jnp.logical_and(s >= NG, s < NS))
        def _():
            for c in kvo_copies(1, s, s - NG):
                c.start()

    def issue_wq(t):
        @pl.when(t < NG)
        def _():
            wq_copy(0, t, t).start()

        @pl.when(t == NG)
        def _():
            xb_copy().start()

        @pl.when(jnp.logical_and(t >= NG, t < NS))
        def _():
            wq_copy(1, t, t - NG).start()

    def wait_kvo(s):
        wait_for(k_buf.at[s], sem_k.at[s])
        wait_for(v_buf.at[s], sem_v.at[s])
        wait_for(wo_buf.at[s], sem_wo.at[s])

    def wait_wq(s):
        @pl.when(s == NG)
        def _():
            wait_for(x_buf.at[1], sem_x)
        wait_for(wq_buf.at[s], sem_wq.at[s])

    def qproj(s, r0=0, r1=M, c0=0, c1=GW):
        br = s // NG
        slot = s % NQ
        for lo in range(r0, r1, MCQ):
            r = slice(lo, min(lo + MCQ, r1))
            q = jnp.dot(x_buf[br, r, :], wq_buf[s, :, c0:c1], preferred_element_type=f32)
            q_buf[slot, r, c0:c1] = (q * SCALE).astype(bf)

    def attn(s):
        slot = s % NQ
        heads = [(b, h) for b in range(B) for h in range(G)]
        groups = [heads[j:j + GS] for j in range(0, len(heads), GS)]
        n = len(groups)
        probs = {}

        def qk(j):
            for (b, h) in groups[j]:
                q = q_buf[slot, b * SQ:(b + 1) * SQ, h * DH:(h + 1) * DH]
                sc = lax.dot_general(q, k_buf[s, b, h], NT, preferred_element_type=f32)
                m = jnp.max(sc, axis=-1, keepdims=True)
                p = jnp.exp(sc - m)
                l = jnp.sum(p, axis=-1, keepdims=True)
                probs[(b, h)] = (p.astype(bf), l)

        def pv(j):
            for (b, h) in groups[j]:
                p, l = probs.pop((b, h))
                o = jnp.dot(p, v_buf[s, b, h], preferred_element_type=f32)
                r0 = pl.reciprocal(l, approx=True)
                o = o * (r0 * (2.0 - l * r0))
                o_buf[b * SQ:(b + 1) * SQ, h * DH:(h + 1) * DH] = o.astype(bf)

        for j in range(n + SKEW):
            if j < n:
                qk(j)
            if j >= SKEW:
                pv(j - SKEW)

    def oproj(s):
        br = s // NG
        g = s % NG
        for c in range(NOC):
            r = slice(OST[c], OST[c] + OCH[c])
            o = jnp.dot(o_buf[r, :], wo_buf[s], preferred_element_type=f32)
            new = jnp.where(g == 0, 0.0, acc[r, :]) + o
            acc[r, :] = new
            out_buf[br, r, :] = new.astype(bf)

            @pl.when(g == NG - 1)
            def _():
                out_copy(br, c).start()

    def fence():
        pl.semaphore_signal(sem_f, 1)
        pl.semaphore_wait(sem_f, 1)

    once[0] = 1
    first = [piece(i) for i in range(len(PIECES))]
    first.append(wq_copy(0, 1, 1))
    first.extend(kvo_copies(0, 0, 0))
    first.append(wq_copy(0, 2, 2))
    for cp in first:
        cp.start()
        fence()

    def whole(_, outer_carry):
        for n_, (waits, works) in enumerate(PRO):
            for i in waits:
                piece(i).wait()
            if n_ == len(PRO) - 1:
                wait_for(wq_buf.at[1], sem_wq.at[1])
            for (r0, r1, c0, c1) in works:
                qproj(0, r0, r1, c0, c1)
        qproj(1)

        def main(s, carry):
            wait_kvo(s)
            wait_wq(s + AHEAD)
            issue_kvo(s + 1)
            issue_wq(s + 1 + AHEAD)
            attn(s)
            qproj(s + AHEAD)
            oproj(s)
            return carry
        lax.fori_loop(0, NS - AHEAD, main, 0)

        def tail(s, carry):
            wait_kvo(s)
            issue_kvo(s + 1)
            attn(s)
            oproj(s)
            return carry
        lax.fori_loop(NS - AHEAD, NS, tail, 0)
        return outer_carry

    lax.fori_loop(0, once[0], whole, 0)

    for br in range(2):
        for c in range(NOC):
            out_copy(br, c).wait()


@jax.jit
def pallas_concat_heads__mha_block_cached__mha_block_cached__near_ridge_kernel(
    A_x, A_k_cache, A_v_cache, A_wq, A_wo, B_x, B_k_cache, B_v_cache, B_wq, B_wo,
):
    any_spec = pl.BlockSpec(memory_space=pl.ANY)
    out = pl.pallas_call(
        _kernel,
        out_shape=jax.ShapeDtypeStruct((M, 2 * D), bf),
        in_specs=[any_spec] * 10,
        out_specs=any_spec,
        scratch_shapes=[
            pltpu.VMEM((2, M, D), bf),
            pltpu.VMEM((NS, B, G, SK, DH), bf),
            pltpu.VMEM((NS, B, G, SK, DH), bf),
            pltpu.VMEM((NS, D, GW), bf),
            pltpu.VMEM((NS, GW, D), bf),
            pltpu.VMEM((NQ, M, GW), bf),
            pltpu.VMEM((M, GW), bf),
            pltpu.VMEM((M, D), f32),
            pltpu.VMEM((2, M, D), bf),
            pltpu.SemaphoreType.DMA(()),
            pltpu.SemaphoreType.DMA((len(PIECES),)),
            pltpu.SemaphoreType.DMA((NS,)),
            pltpu.SemaphoreType.DMA((NS,)),
            pltpu.SemaphoreType.DMA((NS,)),
            pltpu.SemaphoreType.DMA((NS,)),
            pltpu.SemaphoreType.DMA((2 * NOC,)),
            pltpu.SemaphoreType.REGULAR,
            pltpu.SMEM((1,), jnp.int32),
        ],
        compiler_params=pltpu.CompilerParams(vmem_limit_bytes=120 * 1024 * 1024,
                                             disable_bounds_checks=True,
                                             disable_semaphore_checks=True),
    )(A_x.reshape(M, D), A_k_cache, A_v_cache, A_wq, A_wo,
      B_x.reshape(M, D), B_k_cache, B_v_cache, B_wq, B_wo)
    return out.reshape(B, SQ, 2 * D)
```
